```python
import os as _os
_os.environ.setdefault("JAX_PLATFORMS", "cpu")
import jax
import jax.numpy as jnp

def _softmax(x, axis=-1):
    return jax.nn.softmax(x, axis=axis)
def _gelu(x):
    return jax.nn.gelu(x, approximate=True)
def _silu(x):
    return jax.nn.silu(x)
def _sigmoid(x):
    return jax.nn.sigmoid(x)
def _layernorm(x, axis=-1, eps=1e-5):
    m = jnp.mean(x, axis=axis, keepdims=True)
    v = jnp.var(x, axis=axis, keepdims=True)
    return (x - m) / jnp.sqrt(v + eps)
def _scatter_add(tgt, idx, src, axis=0):
    return tgt.at[idx].add(src)
def _segment_sum(src, seg, n):
    return jax.ops.segment_sum(src, seg, n)
class _Rng:
    def __init__(self, key):
        self._k = key
    def _next(self):
        self._k, sub = jax.random.split(self._k)
        return sub
    def normal(self, shape):
        return jax.random.normal(self._next(), shape, dtype=jnp.bfloat16)
    def randint(self, lo, hi, shape):
        return jax.random.randint(self._next(), shape, lo, hi, dtype=jnp.int32)
    def uniform(self, shape, lo=0.0, hi=1.0):
        return jax.random.uniform(self._next(), shape, jnp.bfloat16, lo, hi)
    def permutation(self, n):
        return jax.random.permutation(self._next(), n)


kernel_name = 'sequential_preLN__softmax_full_mha__dense_activation_gelu__prompt'

def setup_inputs():
    _rng = _Rng(jax.random.key(int.from_bytes(__import__("os").urandom(4), "little")))
    _w = (lambda a: (lambda t: t.astype(jnp.bfloat16) if jnp.issubdtype(t.dtype, jnp.floating) else t)(jnp.asarray(a)))
    def _A_setup():
        B, S, D = 1, 2048, 640
        return {
            "x": _w((lambda *s: _rng.normal(s) * 0.05)(B, S, D)),
            "wqkv": _w((lambda *s: _rng.normal(s) * 0.05)(D, 3 * D)),
            "wo": _w((lambda *s: _rng.normal(s) * 0.05)(D, D)),
        }
    _A_in = _A_setup()

    def _B_setup():
        B, S, D, F = 1, 2048, 640, 1536
        return {
            "x": _w((lambda *s: _rng.normal(s) * 0.05)(B, S, D)),
            "w1": _w((lambda *s: _rng.normal(s) * 0.4)(D, F) * (D ** -0.5)),
            "b1": _w((lambda *s: _rng.normal(s) * 0.4)(F) * 0.01),
            "w2": _w((lambda *s: _rng.normal(s) * 0.4)(F, D) * (F ** -0.5)),
            "b2": _w((lambda *s: _rng.normal(s) * 0.05)(D) * 0.01),
        }
    _B_in = _B_setup()

    return {
        "A_x": _A_in["x"],
        "A_wqkv": _A_in["wqkv"],
        "A_wo": _A_in["wo"],
        "B_x": _B_in["x"],
        "B_w1": _B_in["w1"],
        "B_b1": _B_in["b1"],
        "B_w2": _B_in["w2"],
        "B_b2": _B_in["b2"],
    }

def reference(A_x, A_wqkv, A_wo, B_x, B_w1, B_b1, B_w2, B_b2):
    def _A_ref(x, wqkv, wo):
        B, S, D = x.shape
        H = 32; Dh = D // H
        qkv = (lambda x, *d: x.transpose(*d))((x @ wqkv).reshape(B, S, 3, H, Dh), 2, 0, 3, 1, 4)
        q, k, v = qkv[0], qkv[1], qkv[2]
        scale = Dh ** -0.5
        scores = jnp.einsum("bhqd,bhkd->bhqk", q, k) * scale
        p = _softmax(scores, axis=-1)
        o = jnp.einsum("bhqk,bhkd->bhqd", p, v)
        return (lambda x, *d: x.transpose(*d))(o, 0, 2, 1, 3).reshape(B, S, D) @ wo

    def _B_ref(x, w1, b1, w2, b2):
        h = jnp.einsum("bsd,df->bsf", x, w1) + b1
        h = _gelu(h)
        return jnp.einsum("bsf,fd->bsd", h, w2) + b2

    x = A_x
    h = x + _A_ref(_layernorm(x, axis=-1), A_wqkv, A_wo)
    h2 = h + _B_ref(_layernorm(h, axis=-1), B_w1, B_b1, B_w2, B_b2)
    return h2
```

```python
import math

import jax
import jax.numpy as jnp
from jax import lax
import jax.experimental.pallas as pl
import jax.experimental.pallas.tpu as pltpu

S = 2048
D = 640
H = 32
DH = 20
F = 1536
G = 6
NG = 6
VR = 24
TQ = 512
TK = 256
NQ = S // TQ
NC = S // TK
NITEMS = H * NQ
TR1 = 256
TR3 = 256
EPS = 1e-5
QSCALE = (DH ** -0.5) * math.log2(math.e)


def _layernorm(x):
    m = jnp.mean(x, axis=-1, keepdims=True)
    xc = x - m
    v = jnp.mean(xc * xc, axis=-1, keepdims=True)
    return xc * lax.rsqrt(v + EPS)


def _kernel(x_ref, wk_ref, wqvt_ref, wo_ref, w1_ref, b1_ref, w2_ref, b2_ref,
            out_ref, k_s, qt_s, vt_s, ot_s, sbuf0, sbuf1):
    f32 = jnp.float32
    bf16 = jnp.bfloat16

    vrow = lax.broadcasted_iota(jnp.int32, (H * VR, TR1), 0) % VR

    def proj(i, carry):
        r0 = pl.multiple_of(i * TR1, TR1)
        xn = _layernorm(x_ref[pl.ds(r0, TR1), :].astype(f32)).astype(bf16)
        k = jnp.dot(xn, wk_ref[...], preferred_element_type=f32).astype(bf16)
        for g in range(NG):
            k_s[g, pl.ds(r0, TR1), :] = k[:, g * 128:(g + 1) * 128]
        qv = lax.dot_general(wqvt_ref[...], xn, (((1,), (1,)), ((), ())),
                             preferred_element_type=f32)
        qt_s[:, pl.ds(r0, TR1)] = qv[:NG * 128] * QSCALE
        vt_s[:, pl.ds(r0, TR1)] = jnp.where(vrow == DH, 1.0, qv[NG * 128:])
        return carry

    lax.fori_loop(0, S // TR1, proj, None)

    rows = lax.broadcasted_iota(jnp.int32, (128, TQ), 0)

    def step(t, m_prev, wbuf, rbuf, do_a=True, do_b=True):
        if do_a:
            h = t // NQ
            qb = t % NQ
            g = h // G
            lo = (h % G) * DH
            qt = qt_s[pl.ds(pl.multiple_of(g * 128, 128), 128),
                      pl.ds(pl.multiple_of(qb * TQ, TQ), TQ)]
            qm = jnp.where((rows >= lo) & (rows < lo + DH), qt, 0.0).astype(bf16)
            mrun = None
        if do_b:
            tp = t - 1
            hp = tp // NQ
            qbp = tp % NQ
            vr0 = pl.multiple_of(hp * VR, 8)
            acc = jnp.zeros((VR, TQ), f32)
        for c in range(NC):
            if do_a:
                kc = k_s[g, pl.ds(c * TK, TK), :]
                s = jnp.dot(kc, qm, preferred_element_type=f32)
                wbuf[pl.ds(c * TK, TK), :] = s
                mc = jnp.max(s.reshape(TK // 8, 8, TQ), axis=0)
                mrun = mc if mrun is None else jnp.maximum(mrun, mc)
            if do_b:
                sp = rbuf[pl.ds(c * TK, TK), :]
                p = jnp.exp2(sp.reshape(TK // 8, 8, TQ) - m_prev[None]).reshape(TK, TQ)
                vt = vt_s[pl.ds(vr0, VR), pl.ds(c * TK, TK)]
                acc = acc + jnp.dot(vt, p, preferred_element_type=f32)
        m = None
        if do_a:
            m = jnp.broadcast_to(jnp.max(mrun, axis=0, keepdims=True), (8, TQ))
        if do_b:
            l = acc[DH:DH + 1, :]
            ot_s[pl.ds(vr0, VR), pl.ds(pl.multiple_of(qbp * TQ, TQ), TQ)] = acc * (1.0 / l)
        return m

    m0 = step(0, None, sbuf0, sbuf1, do_b=False)

    def body(i, m):
        t = 2 * i + 1
        m = step(t, m, sbuf1, sbuf0)
        m = step(t + 1, m, sbuf0, sbuf1)
        return m

    m = lax.fori_loop(0, NITEMS // 2 - 1, body, m0)
    m = step(NITEMS - 1, m, sbuf1, sbuf0)
    step(NITEMS, m, sbuf0, sbuf1, do_a=False)

    b1 = b1_ref[...].astype(f32)
    b2 = b2_ref[...].astype(f32)

    def tail(i, carry):
        r0 = pl.multiple_of(i * TR3, TR3)
        o = ot_s[:, pl.ds(r0, TR3)].T.astype(bf16)
        attn = jnp.dot(o, wo_ref[...], preferred_element_type=f32)
        h = x_ref[pl.ds(r0, TR3), :].astype(f32) + attn
        hn = _layernorm(h).astype(bf16)
        u = jnp.dot(hn, w1_ref[...], preferred_element_type=f32) + b1
        u = jax.nn.gelu(u, approximate=True).astype(bf16)
        y = jnp.dot(u, w2_ref[...], preferred_element_type=f32) + b2
        out_ref[pl.ds(r0, TR3), :] = (h + y).astype(out_ref.dtype)
        return carry

    lax.fori_loop(0, S // TR3, tail, None)


def _group_cols(w):
    w = jnp.pad(w, ((0, 0), (0, NG * G * DH - H * DH)))
    w = w.reshape(D, NG, G * DH)
    w = jnp.pad(w, ((0, 0), (0, 0), (0, 128 - G * DH)))
    return w.reshape(D, NG * 128)


@jax.jit
def pallas_sequential_preLN__softmax_full_mha__dense_activation_gelu__prompt_kernel(
    A_x: jax.Array,
    A_wqkv: jax.Array,
    A_wo: jax.Array,
    B_x: jax.Array,
    B_w1: jax.Array,
    B_b1: jax.Array,
    B_w2: jax.Array,
    B_b2: jax.Array,
):
    del B_x
    x = A_x.reshape(S, D)
    wq = A_wqkv[:, :D]
    wk = A_wqkv[:, D:2 * D]
    wv = A_wqkv[:, 2 * D:]
    wk_p = _group_cols(wk)
    wqt_p = _group_cols(wq).T
    wvt_p = jnp.pad(wv.T.reshape(H, DH, D), ((0, 0), (0, VR - DH), (0, 0))).reshape(H * VR, D)
    wqvt = jnp.concatenate([wqt_p, wvt_p], axis=0)
    wo_p = jnp.pad(A_wo.reshape(H, DH, D), ((0, 0), (0, VR - DH), (0, 0))).reshape(H * VR, D)

    out = pl.pallas_call(
        _kernel,
        out_shape=jax.ShapeDtypeStruct((S, D), A_x.dtype),
        scratch_shapes=[
            pltpu.VMEM((NG, S, 128), jnp.bfloat16),
            pltpu.VMEM((NG * 128, S), jnp.float32),
            pltpu.VMEM((H * VR, S), jnp.float32),
            pltpu.VMEM((H * VR, S), jnp.float32),
            pltpu.VMEM((S, TQ), jnp.float32),
            pltpu.VMEM((S, TQ), jnp.float32),
        ],
        compiler_params=pltpu.CompilerParams(vmem_limit_bytes=100 * 1024 * 1024),
    )(x, wk_p, wqvt, wo_p, B_w1, B_b1.reshape(1, F), B_w2, B_b2.reshape(1, D))
    return out.reshape(A_x.shape)
```

```python
import math

import jax
import jax.numpy as jnp
from jax import lax
import jax.experimental.pallas as pl
import jax.experimental.pallas.tpu as pltpu

S = 2048
D = 640
H = 32
DH = 20
F = 1536
NB = D // 128
VR = 24
TQ = 512
TK = 128
NQ = S // TQ
QT = TQ // 128
NQT = S // 128
NCA = S // TK - 1
SM = NCA * TK
NVT = NQ * QT
NSL = NQ * NCA
V_LATE = 1
V_EARLY = 6
XC = 256
NXC = S // XC
TR1 = 512
TR3 = 256
NT3 = S // TR3
EPS = 1e-5
QSCALE = (DH ** -0.5) * math.log2(math.e)

SEM_X = 0
SEM_WK = NXC
SEM_WQ = NXC + 1
SEM_WV = NXC + 2
SEM_WO = NXC + 3
SEM_W1 = NXC + 4
SEM_W2 = NXC + 5
SEM_OUT = NXC + 6
NSEM = SEM_OUT + NT3


def _layernorm(x):
    m = jnp.mean(x, axis=-1, keepdims=True)
    xc = x - m
    v = jnp.mean(xc * xc, axis=-1, keepdims=True)
    return xc * lax.rsqrt(v + EPS)


def _kernel(x_hbm, wqkv_hbm, wo_hbm, w1_hbm, b1_ref, w2_hbm, b2_ref, out_hbm,
            x_s, wq_s, wk_s, wv_s, wo_s, w1_s, w2_s, wqvt_s, xn_s,
            k_s, q3_s, vt_s, ot_s, sbuf0, sbuf1, kops, hres_s, hn_s, out_s, zero_s, sems):
    f32 = jnp.float32
    bf16 = jnp.bfloat16

    def x_copy(i):
        return pltpu.make_async_copy(x_hbm.at[0, pl.ds(i * XC, XC), :],
                                     x_s.at[pl.ds(i * XC, XC), :], sems.at[SEM_X + i])

    def w_copy(part, dst, sem):
        return pltpu.make_async_copy(wqkv_hbm.at[:, pl.ds(part * D, D)], dst, sems.at[sem])

    wk_copy = w_copy(1, wk_s, SEM_WK)
    wq_copy = w_copy(0, wq_s, SEM_WQ)
    wv_copy = w_copy(2, wv_s, SEM_WV)
    wo_copy = pltpu.make_async_copy(wo_hbm, wo_s, sems.at[SEM_WO])
    w1_copy = pltpu.make_async_copy(w1_hbm, w1_s, sems.at[SEM_W1])
    w2_copy = pltpu.make_async_copy(w2_hbm, w2_s, sems.at[SEM_W2])

    x_copy(0).start()
    x_copy(1).start()
    wk_copy.start()

    def ln_chunk(i):
        xn_s[i * XC:(i + 1) * XC, :] = _layernorm(
            x_s[i * XC:(i + 1) * XC, :].astype(f32)).astype(bf16)

    lane = lax.broadcasted_iota(jnp.int32, (XC, 128), 1)

    def k_chunk(i):
        r = slice(i * XC, (i + 1) * XC)
        k = jnp.dot(xn_s[r, :], wk_s[...], preferred_element_type=f32)
        for b in range(NB):
            k_s[b, r, :] = k[:, b * 128:(b + 1) * 128].astype(bf16)
        for b in range(NB - 1):
            k_s[NB + b, r, :] = jnp.where(
                lane >= 64, k[:, b * 128:(b + 1) * 128],
                k[:, (b + 1) * 128:(b + 2) * 128]).astype(bf16)

    for i in range(NVT):
        zero_s[i] = 0
    sub = lax.broadcasted_iota(jnp.int32, (8, S), 0)
    tail_rows = jnp.where(sub == DH - 16, 1.0, 0.0).astype(f32)
    for h in range(H):
        vt_s[h * VR + 16:h * VR + 24, :] = tail_rows

    x_copy(0).wait()
    for i in range(2, NXC):
        x_copy(i).start()
    ln_chunk(0)
    x_copy(1).wait()
    ln_chunk(1)
    wk_copy.wait()
    wq_copy.start()
    wv_copy.start()
    k_chunk(0)
    x_copy(2).wait()
    x_copy(3).wait()
    k_chunk(1)
    ln_chunk(2)
    k_chunk(2)
    ln_chunk(3)
    for i in range(4, NXC):
        x_copy(i).wait()
    for i in range(3, NXC - 1):
        k_chunk(i)
        ln_chunk(i + 1)
    wq_copy.wait()
    wv_copy.wait()
    wo_copy.start()
    w1_copy.start()
    w2_copy.start()
    k_chunk(NXC - 1)
    wqvt_s[0:D, :] = wq_s[...].T
    wqvt_s[D:2 * D, :] = wv_s[...].T

    def proj(i, carry):
        r0 = pl.multiple_of(i * TR1, TR1)
        qv = lax.dot_general(wqvt_s[...], xn_s[pl.ds(r0, TR1), :],
                             (((1,), (1,)), ((), ())), preferred_element_type=f32)
        for t in range(TR1 // 128):
            q3_s[i * (TR1 // 128) + t] = qv[:D, t * 128:(t + 1) * 128] * QSCALE
        for h in range(H):
            vt_s[h * VR:h * VR + DH, pl.ds(r0, TR1)] = qv[D + h * DH:D + (h + 1) * DH]
        return carry

    lax.fori_loop(0, S // TR1, proj, None)

    rows = lax.broadcasted_iota(jnp.int32, (128, TQ), 0)
    bufs = (sbuf0, sbuf1)

    def head_geom(h):
        f0 = h * DH + h // 1000003
        b_lo = f0 // 128
        b_hi = (f0 + DH - 1) // 128
        lo = f0 % 128
        kb = jnp.where(b_hi == b_lo, b_lo, NB + b_lo)
        return f0, b_lo, b_hi, lo, kb

    def gen(h):
        _, _, _, lo, kb = head_geom(h)
        kx = k_s[kb, SM:S, :].astype(f32)
        kx = pltpu.roll(kx, (128 - lo) % 128, axis=1)
        for d in range(DH):
            kops[d] = jnp.broadcast_to(kx[:, d:d + 1], (TK, 128))

    def vtile(h, n):
        f0 = h * DH
        z = zero_s[n] + h // 1000003
        acc = None
        for d in range(DH):
            q = q3_s[n, pl.ds(f0 + d + z, 8, stride=0), :]
            term = kops[z + d].reshape(TK // 8, 8, 128) * q[None]
            acc = term if acc is None else acc + term
        m = jnp.max(jnp.max(acc, axis=0), axis=0, keepdims=True)
        p = jnp.exp2(acc - m[None]).reshape(TK, 128)
        vt = vt_s[pl.ds(pl.multiple_of(h * VR, 8), VR), SM:S]
        return m, jnp.dot(vt, p, preferred_element_type=f32)

    def vmerge(vres, qb):
        vm = jnp.concatenate([vres[qb * QT + t][0] for t in range(QT)], axis=1)
        va = jnp.concatenate([vres[qb * QT + t][1] for t in range(QT)], axis=1)
        return vm, va

    def step(h, qb, hp, qbp, m_prev, vprev, vres, par, do_a=True, do_b=True):
        wbuf = bufs[par]
        rbuf = bufs[1 - par]
        if do_a:
            _, b_lo, b_hi, lo, kb = head_geom(h)
            top = pl.ds(pl.multiple_of(b_hi * 128, 128), 64)
            bot = pl.ds(pl.multiple_of(b_lo * 128 + 64, 64), 64)
            qt = jnp.concatenate(
                [jnp.concatenate([q3_s[qb * QT + t, top, :], q3_s[qb * QT + t, bot, :]], axis=0)
                 for t in range(QT)], axis=1)
            qm = jnp.where(((rows - lo) & 127) < DH, qt, 0.0).astype(bf16)
        if do_b:
            vr0 = pl.multiple_of(hp * VR, 8)
        mrun = None
        acc = None
        for c in range(NCA):
            if do_a:
                kc = k_s[kb, c * TK:(c + 1) * TK, :]
                s = jnp.dot(kc, qm, preferred_element_type=f32)
                wbuf[c * TK:(c + 1) * TK, :] = s
                mc = jnp.max(s.reshape(TK // 8, 8, TQ), axis=0)
                mrun = mc if mrun is None else jnp.maximum(mrun, mc)
            if do_b:
                sp = rbuf[c * TK:(c + 1) * TK, :]
                p = jnp.exp2(sp.reshape(TK // 8, 8, TQ) - m_prev[None]).reshape(TK, TQ)
                vt = vt_s[pl.ds(vr0, VR), c * TK:(c + 1) * TK]
                pv = jnp.dot(vt, p, preferred_element_type=f32)
                acc = pv if acc is None else acc + pv
            if do_a:
                slot = qb * NCA + c
                target = 0 if slot < V_LATE else min(
                    NVT, 1 + (slot - V_LATE) * (NVT - 1) // (NSL - 1 - V_LATE - V_EARLY))
                while len(vres) < target:
                    vres.append(vtile(h, len(vres)))
        m = None
        if do_a:
            m = jnp.broadcast_to(jnp.max(mrun, axis=0, keepdims=True), (8, TQ))
        if do_b:
            vm, va = vprev if vprev is not None else vmerge(vres, qbp)
            ma = m_prev[0:1]
            mm = jnp.maximum(ma, vm)
            acc = acc * jnp.exp2(ma - mm) + va * jnp.exp2(vm - mm)
            l = acc[DH:DH + 1, :]
            ot_s[pl.ds(vr0, VR), qbp * TQ:(qbp + 1) * TQ] = acc * (1.0 / l)
        return m

    def head(h, carry, first=False):
        vres = []
        m = None if first else carry[0]
        for qb in range(NQ):
            if qb == 0:
                m = step(h, 0, h - 1, NQ - 1, m, None if first else carry[1:], vres, 0,
                         do_b=not first)
            else:
                m = step(h, qb, h, qb - 1, m, None, vres, qb % 2)
        vm, va = vmerge(vres, NQ - 1)
        gen(jnp.minimum(h + 1, H - 1))
        return (m, vm, va)

    gen(0)
    carry = head(0, None, first=True)
    carry = lax.fori_loop(1, H, head, carry)

    wo_copy.wait()
    w1_copy.wait()
    w2_copy.wait()

    def out_copy(i):
        r0 = pl.multiple_of(i * TR3, TR3)
        return pltpu.make_async_copy(out_s.at[pl.ds(r0, TR3), :],
                                     out_hbm.at[0, pl.ds(r0, TR3), :], sems.at[SEM_OUT + i])

    def attn_out(i):
        r0 = pl.multiple_of(i * TR3, TR3)
        ot = jnp.concatenate(
            [ot_s[h * VR:h * VR + DH, pl.ds(r0, TR3)] for h in range(H)], axis=0)
        o = ot.T.astype(bf16)
        attn = jnp.dot(o, wo_s[...], preferred_element_type=f32)
        hres = x_s[pl.ds(r0, TR3), :].astype(f32) + attn
        hres_s[pl.ds(r0, TR3), :] = hres
        hn_s[pl.ds(r0, TR3), :] = _layernorm(hres).astype(bf16)

    def ffn(i, nxt):
        r0 = pl.multiple_of(i * TR3, TR3)
        b1 = b1_ref[...].astype(f32)
        b2 = b2_ref[...].astype(f32)
        hres = hres_s[pl.ds(r0, TR3), :] + b2
        u = jnp.dot(hn_s[pl.ds(r0, TR3), :], w1_s[...], preferred_element_type=f32) + b1
        u = jax.nn.gelu(u, approximate=True).astype(bf16)
        if nxt:
            attn_out(i + 1)
        y = jnp.dot(u, w2_s[...], preferred_element_type=f32)
        out_s[pl.ds(r0, TR3), :] = (hres + y).astype(bf16)
        out_copy(i).start()

    attn_out(0)
    step(H, 0, H - 1, NQ - 1, carry[0], carry[1:], None, 0, do_a=False)

    def tail(i, c):
        ffn(i, True)
        return c

    lax.fori_loop(0, NT3 - 1, tail, None)
    ffn(NT3 - 1, False)
    for i in range(NT3):
        out_copy(i).wait()


@jax.jit
def pallas_sequential_preLN__softmax_full_mha__dense_activation_gelu__prompt_kernel(
    A_x: jax.Array,
    A_wqkv: jax.Array,
    A_wo: jax.Array,
    B_x: jax.Array,
    B_w1: jax.Array,
    B_b1: jax.Array,
    B_w2: jax.Array,
    B_b2: jax.Array,
):
    del B_x
    bf16 = jnp.bfloat16
    f32 = jnp.float32
    any_spec = pl.BlockSpec(memory_space=pl.ANY)
    vmem_spec = pl.BlockSpec(memory_space=pltpu.VMEM)
    return pl.pallas_call(
        _kernel,
        out_shape=jax.ShapeDtypeStruct(A_x.shape, A_x.dtype),
        in_specs=[any_spec, any_spec, any_spec, any_spec, vmem_spec, any_spec, vmem_spec],
        out_specs=any_spec,
        scratch_shapes=[
            pltpu.VMEM((S, D), bf16),
            pltpu.VMEM((D, D), bf16),
            pltpu.VMEM((D, D), bf16),
            pltpu.VMEM((D, D), bf16),
            pltpu.VMEM((D, D), bf16),
            pltpu.VMEM((D, F), bf16),
            pltpu.VMEM((F, D), bf16),
            pltpu.VMEM((2 * D, D), bf16),
            pltpu.VMEM((S, D), bf16),
            pltpu.VMEM((2 * NB - 1, S, 128), bf16),
            pltpu.VMEM((NQT, D, 128), f32),
            pltpu.VMEM((H * VR, S), f32),
            pltpu.VMEM((H * VR, S), f32),
            pltpu.VMEM((SM, TQ), f32),
            pltpu.VMEM((SM, TQ), f32),
            pltpu.VMEM((DH, TK, 128), f32),
            pltpu.VMEM((S, D), f32),
            pltpu.VMEM((S, D), bf16),
            pltpu.VMEM((S, D), bf16),
            pltpu.SMEM((NVT,), jnp.int32),
            pltpu.SemaphoreType.DMA((NSEM,)),
        ],
        compiler_params=pltpu.CompilerParams(vmem_limit_bytes=100 * 1024 * 1024),
    )(A_x, A_wqkv, A_wo, B_w1, B_b1.reshape(1, F), B_w2, B_b2.reshape(1, D))
```

```python
import math

import jax
import jax.numpy as jnp
from jax import lax
import jax.experimental.pallas as pl
import jax.experimental.pallas.tpu as pltpu

S = 2048
D = 640
H = 32
DH = 20
F = 1536
NB = D // 128
VR = 24
QR = 32
TQ = 512
TK = 128
NQ = S // TQ
QT = TQ // 128
NQT = S // 128
NC = S // TK
NK = 2
NCA = NC - NK
TILES = tuple((kt, t) for kt in reversed(range(NK)) for t in range(NQT))
NVT = len(TILES)
NSL = NQ * NCA
NPB = 4
V_LATE = 2
V_EARLY = 12
XC = 256
NXC = S // XC
TR1 = 1024
TR3 = 256
NT3 = S // TR3
EPS = 1e-5
QSCALE = (DH ** -0.5) * math.log2(math.e)
L_LO = 2.0 ** -20
L_HI = 2.0 ** 80
ACC_HI = 2.0 ** 120

SEM_X = 0
SEM_WK = NXC
SEM_WQ = NXC + 1
SEM_WV = NXC + 2
SEM_WO = NXC + 3
SEM_W1 = NXC + 4
SEM_W2 = NXC + 5
SEM_B1 = NXC + 6
SEM_B2 = NXC + 7
SEM_OUT = NXC + 8
NSEM = SEM_OUT + NT3


def _zero_after(x, n):
    if n == 0:
        return 0
    for i in range(n):
        x = x // (1000003 + i)
    return x


def _layernorm(x):
    m = jnp.mean(x, axis=-1, keepdims=True)
    xc = x - m
    v = jnp.mean(xc * xc, axis=-1, keepdims=True)
    return xc * lax.rsqrt(v + EPS)


def _kernel(x_hbm, wqkv_hbm, wo_hbm, w1_hbm, b1_hbm, w2_hbm, b2_hbm, out_hbm,
            x_s, wq_s, wk_s, wv_s, wo_s, w1_s, w2_s, wqvt_s, xn_s,
            k_s, q3_s, q4_s, vt_s, ot_s, sbuf, kops0, kops1, pb0, pb1, pb2, pb3,
            qm0, qm1, qm2, qm3, zacc_s, pcar_s, acar_s, bad_s, hres_s, hn_s, out_s,
            b1f_s, b2f_s, b1_s, b2_s, zero_s, sems):
    f32 = jnp.float32
    bf16 = jnp.bfloat16
    kops = (kops0, kops1)
    pbs = (pb0, pb1, pb2, pb3)
    qms = (qm0, qm1, qm2, qm3)

    def x_copy(i):
        return pltpu.make_async_copy(x_hbm.at[0, pl.ds(i * XC, XC), :],
                                     x_s.at[pl.ds(i * XC, XC), :], sems.at[SEM_X + i])

    def w_copy(part, dst, sem):
        return pltpu.make_async_copy(wqkv_hbm.at[:, pl.ds(part * D, D)], dst, sems.at[sem])

    wk_copy = w_copy(1, wk_s, SEM_WK)
    wq_copy = w_copy(0, wq_s, SEM_WQ)
    wv_copy = w_copy(2, wv_s, SEM_WV)
    late_copies = (
        pltpu.make_async_copy(wo_hbm, wo_s, sems.at[SEM_WO]),
        pltpu.make_async_copy(w1_hbm, w1_s, sems.at[SEM_W1]),
        pltpu.make_async_copy(w2_hbm, w2_s, sems.at[SEM_W2]),
        pltpu.make_async_copy(b1_hbm, b1_s, sems.at[SEM_B1]),
        pltpu.make_async_copy(b2_hbm, b2_s, sems.at[SEM_B2]),
    )

    x_copy(0).start()
    wk_copy.start()

    rows = lax.broadcasted_iota(jnp.int32, (128, TQ), 0)

    def head_geom(h, depth=1):
        f0 = h * DH + _zero_after(h, depth)
        b_lo = f0 // 128
        b_hi = (f0 + DH - 1) // 128
        lo = f0 % 128
        kb = jnp.where(b_hi == b_lo, b_lo, NB + b_lo)
        return b_lo, b_hi, lo, kb

    def masked_q(h, qb):
        b_lo, b_hi, lo, _ = head_geom(h)
        top = pl.ds(pl.multiple_of(b_hi * 128, 128), 64)
        bot = pl.ds(pl.multiple_of(b_lo * 128 + 64, 64), 64)
        qt = jnp.concatenate(
            [jnp.concatenate([q3_s[qb * QT + t, top, :], q3_s[qb * QT + t, bot, :]], axis=0)
             for t in range(QT)], axis=1)
        return jnp.where(((rows - lo) & 127) < DH, qt, 0.0).astype(bf16)

    def qprep(h, qb):
        qms[qb][0] = pltpu.bitcast(masked_q(h, qb), jnp.uint32)

    def k_rows(kb, k0, n):
        return k_s[kb, k0 // 2:(k0 + n) // 2, :]

    def gen(h, kt):
        _, _, lo, kb = head_geom(h)
        kx = pltpu.bitcast(k_rows(kb, (NC - 1 - kt) * TK, TK), bf16).astype(f32)
        kx = pltpu.roll(kx, (128 - lo) % 128, axis=1)
        for d in range(DH):
            kops[kt][d] = jnp.broadcast_to(kx[:, d:d + 1], (TK, 128))

    def ln_chunk(i):
        xn_s[i * XC:(i + 1) * XC, :] = _layernorm(
            x_s[i * XC:(i + 1) * XC, :].astype(f32)).astype(bf16)

    lane = lax.broadcasted_iota(jnp.int32, (XC // 2, 128), 1)

    def k_part(i, b0, b1):
        k = jnp.dot(xn_s[i * XC:(i + 1) * XC, :], wk_s[:, b0 * 128:b1 * 128],
                    preferred_element_type=f32).astype(bf16)
        k = pltpu.bitcast(k, jnp.uint32)
        r = slice(i * XC // 2, (i + 1) * XC // 2)
        for b in range(b0, b1):
            kb = k[:, (b - b0) * 128:(b - b0 + 1) * 128]
            k_s[b, r, :] = kb
            if b < NB - 1:
                pltpu.store(k_s.at[NB + b, r, :], kb, mask=lane >= 64)
            if b > 0:
                pltpu.store(k_s.at[NB + b - 1, r, :], kb, mask=lane < 64)

    def k_lo(i):
        k_part(i, 0, 2)

    def k_hi(i):
        k_part(i, 2, NB)

    def k_all(i):
        k_part(i, 0, NB)

    def proj(i, carry):
        r0 = pl.multiple_of(i * TR1, TR1)
        qv = lax.dot_general(wqvt_s[...], xn_s[pl.ds(r0, TR1), :],
                             (((1,), (1,)), ((), ())), preferred_element_type=f32)
        for t in range(TR1 // 128):
            q = qv[:D, t * 128:(t + 1) * 128] * QSCALE
            q3_s[i * (TR1 // 128) + t] = q
            qz = jnp.concatenate([q, jnp.zeros((16, 128), f32)], axis=0)
            for h in range(H):
                q4_s[i * (TR1 // 128) + t, h * QR:(h + 1) * QR, :] = qz[h * DH:h * DH + QR]
        for h in range(H):
            vt_s[h * VR:h * VR + DH, pl.ds(r0, TR1)] = qv[D + h * DH:D + (h + 1) * DH]
        return carry

    for i in range(NVT + NSL):
        zero_s[i] = 0
    zacc_s[...] = jnp.zeros(zacc_s.shape, f32)
    pcar_s[...] = jnp.ones(pcar_s.shape, f32)
    acar_s[...] = jnp.zeros(acar_s.shape, f32)
    bad_s[...] = jnp.zeros(bad_s.shape, f32)
    sub = lax.broadcasted_iota(jnp.int32, (8, S), 0)
    tail_rows = jnp.where(sub == DH - 16, 1.0, 0.0).astype(f32)
    for h in range(H):
        vt_s[h * VR + 16:h * VR + 24, :] = tail_rows

    x_copy(0).wait()
    x_copy(1).start()
    ln_chunk(0)
    wk_copy.wait()
    x_copy(7).start()
    x_copy(6).start()
    k_lo(0)
    x_copy(1).wait()
    k_hi(0)
    ln_chunk(1)
    k_lo(1)
    x_copy(7).wait()
    x_copy(6).wait()
    for i in (5, 4, 3, 2):
        x_copy(i).start()
    k_hi(1)
    ln_chunk(7)
    k_all(7)
    ln_chunk(6)
    k_lo(6)
    for i in (5, 4, 3, 2):
        x_copy(i).wait()
    wq_copy.start()
    wv_copy.start()
    k_hi(6)
    ln_chunk(5)
    k_all(5)
    for kt in range(NK):
        gen(0, kt)
    ln_chunk(4)
    k_all(4)
    ln_chunk(3)
    k_lo(3)
    wq_copy.wait()
    wv_copy.wait()
    for c in late_copies:
        c.start()
    k_hi(3)
    ln_chunk(2)
    k_all(2)
    wqvt_s[0:D, :] = wq_s[...].T
    wqvt_s[D:2 * D, :] = wv_s[...].T
    lax.fori_loop(0, S // TR1, proj, None)
    qprep(0, 0)

    def vtile(h, n):
        kt, t = TILES[n]
        z = zero_s[n] + _zero_after(h, 2)
        qrow = pl.multiple_of((h + z) * QR, QR)
        acc = None
        for d in range(DH):
            q = jnp.broadcast_to(q4_s[t, pl.ds(qrow + d, 1), :], (8, 128))
            term = kops[kt][z + d].reshape(TK // 8, 8, 128) * q[None]
            acc = term if acc is None else acc + term
        pb = pbs[n % NPB]
        pb[0] = jnp.exp2(acc).reshape(TK, 128)
        vt = vt_s[pl.ds(pl.multiple_of(h * VR, 8), VR), (NC - 1 - kt) * TK:(NC - kt) * TK]
        return jnp.dot(vt, pb[z], preferred_element_type=f32)

    def fin(h, qb, acc):
        l = acc[DH:DH + 1, :]
        ot_s[pl.ds(pl.multiple_of(h * VR, 8), VR), qb * TQ:(qb + 1) * TQ] = acc * (1.0 / l)
        ok = jnp.abs(acc) <= ACC_HI
        bad = jnp.max(jnp.where(ok, 0.0, 1.0).reshape(VR // 8, 8, TQ), axis=0)
        badl = jnp.where((l >= L_LO) & (l <= L_HI), 0.0, 1.0)
        bad_s[qb] = jnp.maximum(bad_s[qb], jnp.maximum(bad, badl))

    def carried(hp):
        vt = vt_s[pl.ds(pl.multiple_of(hp * VR, 8), VR), (NCA - 1) * TK:NCA * TK]
        r = jnp.dot(vt, pcar_s[...], preferred_element_type=f32)
        fin(hp, NQ - 1, acar_s[...] + r)

    def head(h, carry):
        kb0, hp = carry
        _, _, _, kb = head_geom(h)
        hn = jnp.minimum(h + 1, H - 1)
        vr0 = pl.multiple_of(h * VR, 8)
        pend = []
        vres = []
        accs = [None] * NQ

        def pv(qb, c, p):
            vt = vt_s[pl.ds(vr0, VR), c * TK:(c + 1) * TK]
            r = jnp.dot(vt, p, preferred_element_type=f32)
            accs[qb] = (zacc_s[qb] if accs[qb] is None else accs[qb]) + r

        def total(qb):
            acc = accs[qb]
            for kt in range(NK):
                acc = acc + jnp.concatenate(
                    [vres[TILES.index((kt, qb * QT + t))] for t in range(QT)], axis=1)
            return acc

        for qb in range(1, NQ):
            qprep(h, qb)
        for slot in range(NSL):
            qb, c = divmod(slot, NCA)
            kc = pltpu.bitcast(jnp.concatenate(
                [k_rows(kb0 if slot == 0 else kb, c * TK + 16 * i, 16)
                 for i in reversed(range(8))], axis=0), bf16)
            zq = 0 if slot == 0 else zero_s[NVT + slot] + _zero_after(h, 1)
            w = pltpu.bitcast(qms[qb][zq], bf16)
            e = jnp.exp2(jnp.dot(kc, w, preferred_element_type=f32))
            pend.append((qb, c, jnp.concatenate(
                [e[16 * i:16 * (i + 1)] for i in reversed(range(8))], axis=0)))
            if slot == 0:
                carried(hp)
            else:
                pv(*pend.pop(0))
            target = min(NVT, max(0, slot + 1 - V_LATE) * NVT // (NSL - V_LATE - V_EARLY))
            while len(vres) < target:
                vres.append(vtile(h, len(vres)))
                n = len(vres)
                if n == NVT or TILES[n][0] != TILES[n - 1][0]:
                    gen(hn, TILES[n - 1][0])
        pcar_s[...] = pend.pop(0)[2]
        acar_s[...] = total(NQ - 1)
        for qb in range(NQ - 1):
            fin(h, qb, total(qb))
        qprep(hn, 0)
        return head_geom(hn, 0)[3], h

    def out_copy(i):
        r0 = pl.multiple_of(i * TR3, TR3)
        return pltpu.make_async_copy(out_s.at[pl.ds(r0, TR3), :],
                                     out_hbm.at[0, pl.ds(r0, TR3), :], sems.at[SEM_OUT + i])

    def attn_out(i):
        r0 = pl.multiple_of(i * TR3, TR3)
        ot = jnp.concatenate(
            [ot_s[h * VR:h * VR + DH, pl.ds(r0, TR3)] for h in range(H)], axis=0)
        o = ot.T.astype(bf16)
        attn = jnp.dot(o, wo_s[...], preferred_element_type=f32)
        hres = x_s[pl.ds(r0, TR3), :].astype(f32) + attn
        hres_s[pl.ds(r0, TR3), :] = hres
        hn_s[pl.ds(r0, TR3), :] = _layernorm(hres).astype(bf16)

    def ffn(i, with_next):
        r0 = pl.multiple_of(i * TR3, TR3)
        hres = hres_s[pl.ds(r0, TR3), :] + b2f_s[0:1, :]
        u = jnp.dot(hn_s[pl.ds(r0, TR3), :], w1_s[...],
                    preferred_element_type=f32) + b1f_s[0:1, :]
        u = jax.nn.gelu(u, approximate=True).astype(bf16)
        if with_next:
            attn_out(i + 1)
        y = jnp.dot(u, w2_s[...], preferred_element_type=f32)
        out_s[pl.ds(r0, TR3), :] = (hres + y).astype(bf16)
        out_copy(i).start()

    lax.fori_loop(0, H, head, (jnp.int32(0), jnp.int32(H - 1)))
    for c in late_copies:
        c.wait()
    b1f_s[...] = jnp.broadcast_to(b1_s[...].astype(f32).reshape(1, F), (8, F))
    b2f_s[...] = jnp.broadcast_to(b2_s[...].astype(f32).reshape(1, D), (8, D))
    carried(H - 1)
    attn_out(0)

    @pl.when(jnp.max(bad_s[...]) > 0.0)
    def _():
        def item(t, carry):
            h = t // NQ
            qb = t % NQ
            _, _, _, kb = head_geom(h)
            qm = masked_q(h, qb)
            vr0 = pl.multiple_of(h * VR, 8)
            mrun = None
            for c in range(NC):
                kc = pltpu.bitcast(k_rows(kb, c * TK, TK), bf16)
                s = jnp.dot(kc, qm, preferred_element_type=f32)
                sbuf[c * TK:(c + 1) * TK, :] = s
                mc = jnp.max(s.reshape(TK // 8, 8, TQ), axis=0)
                mrun = mc if mrun is None else jnp.maximum(mrun, mc)
            m = jnp.max(mrun, axis=0, keepdims=True)
            acc = None
            for c in range(NC):
                p = jnp.exp2(sbuf[c * TK:(c + 1) * TK, :] - m)
                r = jnp.dot(vt_s[pl.ds(vr0, VR), c * TK:(c + 1) * TK], p,
                            preferred_element_type=f32)
                acc = r if acc is None else acc + r
            l = acc[DH:DH + 1, :]
            ot_s[pl.ds(vr0, VR), pl.ds(pl.multiple_of(qb * TQ, TQ), TQ)] = acc * (1.0 / l)
            return carry

        lax.fori_loop(0, H * NQ, item, None)
        attn_out(0)

    def tail(i, c):
        ffn(i, True)
        return c

    lax.fori_loop(0, NT3 - 1, tail, None)
    ffn(NT3 - 1, False)
    for i in range(NT3):
        out_copy(i).wait()


@jax.jit
def pallas_sequential_preLN__softmax_full_mha__dense_activation_gelu__prompt_kernel(
    A_x: jax.Array,
    A_wqkv: jax.Array,
    A_wo: jax.Array,
    B_x: jax.Array,
    B_w1: jax.Array,
    B_b1: jax.Array,
    B_w2: jax.Array,
    B_b2: jax.Array,
):
    del B_x
    bf16 = jnp.bfloat16
    f32 = jnp.float32
    u32 = jnp.uint32
    any_spec = pl.BlockSpec(memory_space=pl.ANY)
    return pl.pallas_call(
        _kernel,
        out_shape=jax.ShapeDtypeStruct(A_x.shape, A_x.dtype),
        in_specs=[any_spec] * 7,
        out_specs=any_spec,
        scratch_shapes=[
            pltpu.VMEM((S, D), bf16),
            pltpu.VMEM((D, D), bf16),
            pltpu.VMEM((D, D), bf16),
            pltpu.VMEM((D, D), bf16),
            pltpu.VMEM((D, D), bf16),
            pltpu.VMEM((D, F), bf16),
            pltpu.VMEM((F, D), bf16),
            pltpu.VMEM((2 * D, D), bf16),
            pltpu.VMEM((S, D), bf16),
            pltpu.VMEM((2 * NB - 1, S // 2, 128), u32),
            pltpu.VMEM((NQT, D, 128), f32),
            pltpu.VMEM((NQT, H * QR, 128), f32),
            pltpu.VMEM((H * VR, S), f32),
            pltpu.VMEM((H * VR, S), f32),
            pltpu.VMEM((S, TQ), f32),
            pltpu.VMEM((DH, TK, 128), f32),
            pltpu.VMEM((DH, TK, 128), f32),
        ] + [pltpu.VMEM((1, TK, 128), f32)] * NPB
          + [pltpu.VMEM((1, 64, TQ), u32)] * NQ + [
            pltpu.VMEM((NQ, VR, TQ), f32),
            pltpu.VMEM((TK, TQ), f32),
            pltpu.VMEM((VR, TQ), f32),
            pltpu.VMEM((NQ, 8, TQ), f32),
            pltpu.VMEM((S, D), f32),
            pltpu.VMEM((S, D), bf16),
            pltpu.VMEM((S, D), bf16),
            pltpu.VMEM((8, F), f32),
            pltpu.VMEM((8, D), f32),
            pltpu.VMEM((F,), bf16),
            pltpu.VMEM((D,), bf16),
            pltpu.SMEM((NVT + NSL,), jnp.int32),
            pltpu.SemaphoreType.DMA((NSEM,)),
        ],
        compiler_params=pltpu.CompilerParams(vmem_limit_bytes=100 * 1024 * 1024),
    )(A_x, A_wqkv, A_wo, B_w1, B_b1, B_w2, B_b2)
```

```python
import math

import jax
import jax.numpy as jnp
from jax import lax
import jax.experimental.pallas as pl
import jax.experimental.pallas.tpu as pltpu

S = 2048
D = 640
H = 32
DH = 20
F = 1536
NB = D // 128
VR = 24
QR = 32
TQ = 512
TK = 128
NQ = S // TQ
QT = TQ // 128
NQT = S // 128
NC = S // TK
NKS = (2, 3, 2, 2)
NK = max(NKS)
NCA = tuple(NC - k for k in NKS)
TILES = tuple((kt, t) for kt in reversed(range(NK)) for t in range(NQT)
              if NKS[t // QT] > kt)
NVT = len(TILES)
SLOTS = tuple((qb, c) for qb in range(NQ) for c in range(NCA[qb]))
NSL = len(SLOTS)
NPB = 4
V_LATE = 1
V_EARLY = 2
DLINE = {TILES.index((1, 0)) + 9: 2, TILES.index((0, 0)) + 9: 1}
XC = 256
NXC = S // XC
TR1 = 1024
TR3 = 256
NT3 = S // TR3
TAIL = 64
EPS = 1e-5
QSCALE = (DH ** -0.5) * math.log2(math.e)
L_LO = 2.0 ** -20
L_HI = 2.0 ** 80
ACC_HI = 2.0 ** 120

SEM_X = 0
SEM_WK = NXC
SEM_WQ = NXC + 1
SEM_WV = NXC + 2
SEM_WO = NXC + 3
SEM_W1 = NXC + 4
SEM_W2 = NXC + 5
SEM_B1 = NXC + 6
SEM_B2 = NXC + 7
SEM_OUT = NXC + 8
NSEM = SEM_OUT + NT3 + 1


def _zero_after(x, n):
    if n == 0:
        return 0
    for i in range(n):
        x = x // (1000003 + i)
    return x


def _layernorm(x):
    m = jnp.mean(x, axis=-1, keepdims=True)
    xc = x - m
    v = jnp.mean(xc * xc, axis=-1, keepdims=True)
    return xc * lax.rsqrt(v + EPS)


def _kernel(x_hbm, wqkv_hbm, wo_hbm, w1_hbm, b1_hbm, w2_hbm, b2_hbm, out_hbm,
            x_s, wq_s, wk_s, wv_s, wo_s, w1_s, w2_s, wqvt_s, xn_s,
            k_s, q3_s, q4_s, vt_s, ot_s, sbuf, kops0, kops1, kops2, pb0, pb1, pb2, pb3,
            qm0, qm1, qm2, qm3, zacc_s, pcar_s, acar_s, bad_s, hres_s, hn_s, out_s,
            b1f_s, b2f_s, b1_s, b2_s, zero_s, sems):
    f32 = jnp.float32
    bf16 = jnp.bfloat16
    kops = (kops0, kops1, kops2)
    pbs = (pb0, pb1, pb2, pb3)
    qms = (qm0, qm1, qm2, qm3)

    def x_copy(i):
        return pltpu.make_async_copy(x_hbm.at[0, pl.ds(i * XC, XC), :],
                                     x_s.at[pl.ds(i * XC, XC), :], sems.at[SEM_X + i])

    def w_copy(part, dst, sem):
        return pltpu.make_async_copy(wqkv_hbm.at[:, pl.ds(part * D, D)], dst, sems.at[sem])

    wk_copy = w_copy(1, wk_s, SEM_WK)
    wq_copy = w_copy(0, wq_s, SEM_WQ)
    wv_copy = w_copy(2, wv_s, SEM_WV)
    late_copies = (
        pltpu.make_async_copy(wo_hbm, wo_s, sems.at[SEM_WO]),
        pltpu.make_async_copy(w1_hbm, w1_s, sems.at[SEM_W1]),
        pltpu.make_async_copy(w2_hbm, w2_s, sems.at[SEM_W2]),
        pltpu.make_async_copy(b1_hbm, b1_s, sems.at[SEM_B1]),
        pltpu.make_async_copy(b2_hbm, b2_s, sems.at[SEM_B2]),
    )

    x_copy(0).start()
    wk_copy.start()

    rows = 2 * lax.broadcasted_iota(jnp.int32, (64, TQ), 0)

    def head_geom(h, depth=1):
        f0 = h * DH + _zero_after(h, depth)
        b_lo = f0 // 128
        b_hi = (f0 + DH - 1) // 128
        lo = f0 % 128
        kb = jnp.where(b_hi == b_lo, b_lo, NB + b_lo)
        return b_lo, b_hi, lo, kb

    def masked_q(h, qb):
        b_lo, b_hi, lo, _ = head_geom(h)
        top = pl.ds(pl.multiple_of(b_hi * 64, 64), 32)
        bot = pl.ds(pl.multiple_of(b_lo * 64 + 32, 32), 32)
        qt = jnp.concatenate(
            [jnp.concatenate([q3_s[qb * QT + t, top, :], q3_s[qb * QT + t, bot, :]], axis=0)
             for t in range(QT)], axis=1)
        return jnp.where(((rows - lo) & 127) < DH, qt, jnp.uint32(0))

    def qprep(h, qb):
        qms[qb][0] = masked_q(h, qb)

    def k_rows(kb, k0, n):
        return k_s[kb, k0 // 2:(k0 + n) // 2, :]

    def gen(h, kt):
        _, _, lo, kb = head_geom(h)
        kx = pltpu.bitcast(k_rows(kb, (NC - 1 - kt) * TK, TK), bf16).astype(f32)
        kx = pltpu.roll(kx, (128 - lo) % 128, axis=1)
        for d in range(DH):
            kops[kt][d] = jnp.broadcast_to(kx[:, d:d + 1], (TK, 128))

    def ln_chunk(i):
        xn_s[i * XC:(i + 1) * XC, :] = _layernorm(
            x_s[i * XC:(i + 1) * XC, :].astype(f32)).astype(bf16)

    lane = lax.broadcasted_iota(jnp.int32, (XC // 2, 128), 1)

    def k_part(i, b0, b1):
        k = jnp.dot(xn_s[i * XC:(i + 1) * XC, :], wk_s[:, b0 * 128:b1 * 128],
                    preferred_element_type=f32).astype(bf16)
        k = pltpu.bitcast(k, jnp.uint32)
        r = slice(i * XC // 2, (i + 1) * XC // 2)
        for b in range(b0, b1):
            kb = k[:, (b - b0) * 128:(b - b0 + 1) * 128]
            k_s[b, r, :] = kb
            if b < NB - 1:
                pltpu.store(k_s.at[NB + b, r, :], kb, mask=lane >= 64)
            if b > 0:
                pltpu.store(k_s.at[NB + b - 1, r, :], kb, mask=lane < 64)

    def k_lo(i):
        k_part(i, 0, 2)

    def k_hi(i):
        k_part(i, 2, NB)

    def k_all(i):
        k_part(i, 0, NB)

    def proj(i, carry):
        r0 = pl.multiple_of(i * TR1, TR1)
        qv = lax.dot_general(wqvt_s[...], xn_s[pl.ds(r0, TR1), :],
                             (((1,), (1,)), ((), ())), preferred_element_type=f32)
        for t in range(TR1 // 128):
            q = qv[:D, t * 128:(t + 1) * 128] * QSCALE
            q3_s[i * (TR1 // 128) + t] = pltpu.bitcast(q.astype(bf16), jnp.uint32)
            qz = jnp.concatenate([q, jnp.zeros((16, 128), f32)], axis=0)
            for h in range(H):
                q4_s[i * (TR1 // 128) + t, h * QR:(h + 1) * QR, :] = qz[h * DH:h * DH + QR]
        for h in range(H):
            vt_s[h * VR:h * VR + DH, pl.ds(r0, TR1)] = qv[D + h * DH:D + (h + 1) * DH]
        return carry

    for i in range(NVT + NSL):
        zero_s[i] = 0
    zacc_s[...] = jnp.zeros(zacc_s.shape, f32)
    pcar_s[...] = jnp.ones(pcar_s.shape, f32)
    acar_s[...] = jnp.zeros(acar_s.shape, f32)
    bad_s[...] = jnp.zeros(bad_s.shape, f32)
    sub = lax.broadcasted_iota(jnp.int32, (8, S), 0)
    tail_rows = jnp.where(sub == DH - 16, 1.0, 0.0).astype(f32)
    for h in range(H):
        vt_s[h * VR + 16:h * VR + 24, :] = tail_rows

    x_copy(0).wait()
    x_copy(1).start()
    ln_chunk(0)
    wk_copy.wait()
    x_copy(7).start()
    x_copy(6).start()
    k_lo(0)
    x_copy(1).wait()
    k_hi(0)
    ln_chunk(1)
    k_lo(1)
    x_copy(7).wait()
    x_copy(6).wait()
    for i in (5, 4, 3, 2):
        x_copy(i).start()
    k_hi(1)
    ln_chunk(7)
    k_all(7)
    ln_chunk(6)
    k_lo(6)
    for i in (5, 4, 3, 2):
        x_copy(i).wait()
    wq_copy.start()
    wv_copy.start()
    k_hi(6)
    ln_chunk(5)
    k_all(5)
    for kt in range(NK):
        gen(0, kt)
    ln_chunk(4)
    k_all(4)
    ln_chunk(3)
    k_lo(3)
    wq_copy.wait()
    wv_copy.wait()
    for c in late_copies:
        c.start()
    k_hi(3)
    ln_chunk(2)
    k_all(2)
    wqvt_s[0:D, :] = wq_s[...].T
    wqvt_s[D:2 * D, :] = wv_s[...].T
    lax.fori_loop(0, S // TR1, proj, None)
    qprep(0, 0)

    def vtile(h, n):
        kt, t = TILES[n]
        z = zero_s[n] + _zero_after(h, 2)
        qrow = pl.multiple_of((h + z) * QR, QR)
        acc = None
        for d in range(DH):
            q = jnp.broadcast_to(q4_s[t, pl.ds(qrow + d, 1), :], (8, 128))
            term = kops[kt][z + d].reshape(TK // 8, 8, 128) * q[None]
            acc = term if acc is None else acc + term
        pb, o = (kops[DLINE[n]], DH) if n in DLINE else (pbs[n % NPB], 0)
        pb[o] = jnp.exp2(acc).reshape(TK, 128)
        vt = vt_s[pl.ds(pl.multiple_of(h * VR, 8), VR), (NC - 1 - kt) * TK:(NC - kt) * TK]
        return jnp.dot(vt, pb[o + z], preferred_element_type=f32)

    def fin(h, qb, acc):
        l = acc[DH:DH + 1, :]
        ot_s[pl.ds(pl.multiple_of(h * VR, 8), VR), qb * TQ:(qb + 1) * TQ] = acc * (1.0 / l)
        ok = jnp.abs(acc) <= ACC_HI
        bad = jnp.max(jnp.where(ok, 0.0, 1.0).reshape(VR // 8, 8, TQ), axis=0)
        badl = jnp.where((l >= L_LO) & (l <= L_HI), 0.0, 1.0)
        bad_s[qb] = jnp.maximum(bad_s[qb], jnp.maximum(bad, badl))

    def carried(hp):
        vt = vt_s[pl.ds(pl.multiple_of(hp * VR, 8), VR), (NCA[-1] - 1) * TK:NCA[-1] * TK]
        r = jnp.dot(vt, pcar_s[...], preferred_element_type=f32)
        fin(hp, NQ - 1, acar_s[...] + r)

    def head(h, carry):
        kb0, hp = carry
        _, _, _, kb = head_geom(h)
        hn = jnp.minimum(h + 1, H - 1)
        vr0 = pl.multiple_of(h * VR, 8)
        pend = []
        vres = []
        accs = [None] * NQ

        def pv(qb, c, p):
            vt = vt_s[pl.ds(vr0, VR), c * TK:(c + 1) * TK]
            r = jnp.dot(vt, p, preferred_element_type=f32)
            accs[qb] = (zacc_s[qb] if accs[qb] is None else accs[qb]) + r

        def total(qb):
            acc = accs[qb]
            for kt in range(NKS[qb]):
                acc = acc + jnp.concatenate(
                    [vres[TILES.index((kt, qb * QT + t))] for t in range(QT)], axis=1)
            return acc

        for qb in range(1, NQ):
            qprep(h, qb)
        for slot in range(NSL):
            qb, c = SLOTS[slot]
            kc = pltpu.bitcast(jnp.concatenate(
                [k_rows(kb0 if slot == 0 else kb, c * TK + 16 * i, 16)
                 for i in reversed(range(8))], axis=0), bf16)
            zq = 0 if slot == 0 else zero_s[NVT + slot] + _zero_after(h, 1)
            w = pltpu.bitcast(qms[qb][zq], bf16)
            e = jnp.exp2(jnp.dot(kc, w, preferred_element_type=f32))
            pend.append((qb, c, jnp.concatenate(
                [e[16 * i:16 * (i + 1)] for i in reversed(range(8))], axis=0)))
            if slot == 0:
                carried(hp)
            else:
                pv(*pend.pop(0))
            target = min(NVT, max(0, slot + 1 - V_LATE) * NVT // (NSL - V_LATE - V_EARLY))
            while len(vres) < target:
                vres.append(vtile(h, len(vres)))
                n = len(vres)
                if n == NVT or TILES[n][0] != TILES[n - 1][0]:
                    gen(hn, TILES[n - 1][0])
        pcar_s[...] = pend.pop(0)[2]
        acar_s[...] = total(NQ - 1)
        for qb in range(NQ - 1):
            fin(h, qb, total(qb))
        qprep(hn, 0)
        return head_geom(hn, 0)[3], h

    def out_copy(i, r0=None, n=TR3):
        if r0 is None:
            r0 = pl.multiple_of(i * TR3, TR3)
        return pltpu.make_async_copy(out_s.at[pl.ds(r0, n), :],
                                     out_hbm.at[0, pl.ds(r0, n), :], sems.at[SEM_OUT + i])

    LAST = ((NT3 - 1, S - TR3, TR3 - TAIL), (NT3, S - TAIL, TAIL))

    def attn_out(i):
        r0 = pl.multiple_of(i * TR3, TR3)
        ot = jnp.concatenate(
            [ot_s[h * VR:h * VR + DH, pl.ds(r0, TR3)] for h in range(H)], axis=0)
        o = ot.T.astype(bf16)
        attn = jnp.dot(o, wo_s[...], preferred_element_type=f32)
        hres = x_s[pl.ds(r0, TR3), :].astype(f32) + attn
        hres_s[pl.ds(r0, TR3), :] = hres
        hn_s[pl.ds(r0, TR3), :] = _layernorm(hres).astype(bf16)

    def ffn(i, with_next):
        r0 = pl.multiple_of(i * TR3, TR3)
        hres = hres_s[pl.ds(r0, TR3), :] + b2f_s[0:1, :]
        u = jnp.dot(hn_s[pl.ds(r0, TR3), :], w1_s[...],
                    preferred_element_type=f32) + b1f_s[0:1, :]
        u = jax.nn.gelu(u, approximate=True).astype(bf16)
        if with_next:
            attn_out(i + 1)
            y = jnp.dot(u, w2_s[...], preferred_element_type=f32)
            out_s[pl.ds(r0, TR3), :] = (hres + y).astype(bf16)
            out_copy(i).start()
        else:
            for j, a, n in LAST:
                r = slice(a - (S - TR3), a - (S - TR3) + n)
                y = jnp.dot(u[r], w2_s[...], preferred_element_type=f32)
                out_s[a:a + n, :] = (hres[r] + y).astype(bf16)
                out_copy(j, a, n).start()

    lax.fori_loop(0, H, head, (jnp.int32(0), jnp.int32(H - 1)))
    for c in late_copies:
        c.wait()
    b1f_s[...] = jnp.broadcast_to(b1_s[...].astype(f32).reshape(1, F), (8, F))
    b2f_s[...] = jnp.broadcast_to(b2_s[...].astype(f32).reshape(1, D), (8, D))
    carried(H - 1)
    attn_out(0)

    @pl.when(jnp.max(bad_s[...]) > 0.0)
    def _():
        def item(t, carry):
            h = t // NQ
            qb = t % NQ
            _, _, _, kb = head_geom(h)
            qm = pltpu.bitcast(masked_q(h, qb), bf16)
            vr0 = pl.multiple_of(h * VR, 8)
            mrun = None
            for c in range(NC):
                kc = pltpu.bitcast(k_rows(kb, c * TK, TK), bf16)
                s = jnp.dot(kc, qm, preferred_element_type=f32)
                sbuf[c * TK:(c + 1) * TK, :] = s
                mc = jnp.max(s.reshape(TK // 8, 8, TQ), axis=0)
                mrun = mc if mrun is None else jnp.maximum(mrun, mc)
            m = jnp.max(mrun, axis=0, keepdims=True)
            acc = None
            for c in range(NC):
                p = jnp.exp2(sbuf[c * TK:(c + 1) * TK, :] - m)
                r = jnp.dot(vt_s[pl.ds(vr0, VR), c * TK:(c + 1) * TK], p,
                            preferred_element_type=f32)
                acc = r if acc is None else acc + r
            l = acc[DH:DH + 1, :]
            ot_s[pl.ds(vr0, VR), pl.ds(pl.multiple_of(qb * TQ, TQ), TQ)] = acc * (1.0 / l)
            return carry

        lax.fori_loop(0, H * NQ, item, None)
        attn_out(0)

    def tail(i, c):
        ffn(i, True)
        return c

    lax.fori_loop(0, NT3 - 1, tail, None)
    ffn(NT3 - 1, False)
    for i in range(NT3 - 1):
        out_copy(i).wait()
    for j, a, n in LAST:
        out_copy(j, a, n).wait()


@jax.jit
def pallas_sequential_preLN__softmax_full_mha__dense_activation_gelu__prompt_kernel(
    A_x: jax.Array,
    A_wqkv: jax.Array,
    A_wo: jax.Array,
    B_x: jax.Array,
    B_w1: jax.Array,
    B_b1: jax.Array,
    B_w2: jax.Array,
    B_b2: jax.Array,
):
    del B_x
    bf16 = jnp.bfloat16
    f32 = jnp.float32
    u32 = jnp.uint32
    any_spec = pl.BlockSpec(memory_space=pl.ANY)
    return pl.pallas_call(
        _kernel,
        out_shape=jax.ShapeDtypeStruct(A_x.shape, A_x.dtype),
        in_specs=[any_spec] * 7,
        out_specs=any_spec,
        scratch_shapes=[
            pltpu.VMEM((S, D), bf16),
            pltpu.VMEM((D, D), bf16),
            pltpu.VMEM((D, D), bf16),
            pltpu.VMEM((D, D), bf16),
            pltpu.VMEM((D, D), bf16),
            pltpu.VMEM((D, F), bf16),
            pltpu.VMEM((F, D), bf16),
            pltpu.VMEM((2 * D, D), bf16),
            pltpu.VMEM((S, D), bf16),
            pltpu.VMEM((2 * NB - 1, S // 2, 128), u32),
            pltpu.VMEM((NQT, D // 2, 128), u32),
            pltpu.VMEM((NQT, H * QR, 128), f32),
            pltpu.VMEM((H * VR, S), f32),
            pltpu.VMEM((H * VR, S), f32),
            pltpu.VMEM((S, TQ), f32),
            pltpu.VMEM((DH + 1, TK, 128), f32),
            pltpu.VMEM((DH + 1, TK, 128), f32),
            pltpu.VMEM((DH + 1, TK, 128), f32),
        ] + [pltpu.VMEM((1, TK, 128), f32)] * NPB
          + [pltpu.VMEM((1, 64, TQ), u32)] * NQ + [
            pltpu.VMEM((NQ, VR, TQ), f32),
            pltpu.VMEM((TK, TQ), f32),
            pltpu.VMEM((VR, TQ), f32),
            pltpu.VMEM((NQ, 8, TQ), f32),
            pltpu.VMEM((S, D), f32),
            pltpu.VMEM((S, D), bf16),
            pltpu.VMEM((S, D), bf16),
            pltpu.VMEM((8, F), f32),
            pltpu.VMEM((8, D), f32),
            pltpu.VMEM((F,), bf16),
            pltpu.VMEM((D,), bf16),
            pltpu.SMEM((NVT + NSL,), jnp.int32),
            pltpu.SemaphoreType.DMA((NSEM,)),
        ],
        compiler_params=pltpu.CompilerParams(vmem_limit_bytes=100 * 1024 * 1024),
    )(A_x, A_wqkv, A_wo, B_w1, B_b1, B_w2, B_b2)
```

```python
import math

import jax
import jax.numpy as jnp
from jax import lax
import jax.experimental.pallas as pl
import jax.experimental.pallas.tpu as pltpu

S = 2048
D = 640
H = 32
DH = 20
F = 1536
NB = D // 128
VR = 24
QR = 32
TQ = 512
TK = 128
NQ = S // TQ
QT = TQ // 128
NQT = S // 128
NC = S // TK
NKS = (2, 3, 2, 2)
NK = max(NKS)
NCA = tuple(NC - k for k in NKS)
TILES = tuple((kt, t) for kt in reversed(range(NK)) for t in range(NQT)
              if NKS[t // QT] > kt)
NVT = len(TILES)
SLOTS = tuple((qb, c) for qb in range(NQ) for c in range(NCA[qb]))
NSL = len(SLOTS)
NPB = 4
V_LATE = 1
V_EARLY = 2
DLINE = {TILES.index((1, 0)) + 9: 2, TILES.index((0, 0)) + 9: 1}
XC = 256
NXC = S // XC
TR1 = 1024
TR3 = 256
NT3 = S // TR3
TAIL = 64
EPS = 1e-5
QSCALE = (DH ** -0.5) * math.log2(math.e)
L_LO = 2.0 ** -20
L_HI = 2.0 ** 80
ACC_HI = 2.0 ** 120

SEM_X = 0
SEM_WK = NXC
SEM_WQ = NXC + 1
SEM_WV = NXC + 2
SEM_WO = NXC + 3
SEM_W1 = NXC + 4
SEM_W2 = NXC + 5
SEM_B1 = NXC + 6
SEM_B2 = NXC + 7
SEM_OUT = NXC + 8
NSEM = SEM_OUT + NT3 + 1


def _zero_after(x, n):
    if n == 0:
        return 0
    for i in range(n):
        x = x // (1000003 + i)
    return x


def _layernorm(x):
    m = jnp.mean(x, axis=-1, keepdims=True)
    xc = x - m
    v = jnp.mean(xc * xc, axis=-1, keepdims=True)
    return xc * lax.rsqrt(v + EPS)


def _kernel(x_hbm, wqkv_hbm, wo_hbm, w1_hbm, b1_hbm, w2_hbm, b2_hbm, out_hbm,
            x_s, wq_s, wk_s, wv_s, wo_s, w1_s, w2_s, wqvt_s, xn_s,
            k_s, q3_s, q4_s, vt_s, ot_s, sbuf, kops0, kops1, kops2, pb0, pb1, pb2, pb3,
            qm0, qm1, qm2, qm3, zacc_s, pcar_s, acar_s, bad_s, hres_s, hn_s, out_s,
            b1f_s, b2f_s, b1_s, b2_s, sems):
    f32 = jnp.float32
    bf16 = jnp.bfloat16
    kops = (kops0, kops1, kops2)
    pbs = (pb0, pb1, pb2, pb3)
    qms = (qm0, qm1, qm2, qm3)

    def x_copy(i):
        return pltpu.make_async_copy(x_hbm.at[0, pl.ds(i * XC, XC), :],
                                     x_s.at[pl.ds(i * XC, XC), :], sems.at[SEM_X + i])

    def w_copy(part, dst, sem):
        return pltpu.make_async_copy(wqkv_hbm.at[:, pl.ds(part * D, D)], dst, sems.at[sem])

    wk_copy = w_copy(1, wk_s, SEM_WK)
    wq_copy = w_copy(0, wq_s, SEM_WQ)
    wv_copy = w_copy(2, wv_s, SEM_WV)
    late_copies = (
        pltpu.make_async_copy(wo_hbm, wo_s, sems.at[SEM_WO]),
        pltpu.make_async_copy(w1_hbm, w1_s, sems.at[SEM_W1]),
        pltpu.make_async_copy(w2_hbm, w2_s, sems.at[SEM_W2]),
        pltpu.make_async_copy(b1_hbm, b1_s, sems.at[SEM_B1]),
        pltpu.make_async_copy(b2_hbm, b2_s, sems.at[SEM_B2]),
    )

    x_copy(0).start()
    wk_copy.start()

    rows = 2 * lax.broadcasted_iota(jnp.int32, (64, TQ), 0)

    def head_geom(h, depth=1):
        f0 = h * DH + _zero_after(h, depth)
        b_lo = f0 // 128
        b_hi = (f0 + DH - 1) // 128
        lo = f0 % 128
        kb = jnp.where(b_hi == b_lo, b_lo, NB + b_lo)
        return b_lo, b_hi, lo, kb

    def masked_q(h, qb):
        b_lo, b_hi, lo, _ = head_geom(h)
        top = pl.ds(pl.multiple_of(b_hi * 64, 64), 32)
        bot = pl.ds(pl.multiple_of(b_lo * 64 + 32, 32), 32)
        qt = jnp.concatenate(
            [jnp.concatenate([q3_s[qb * QT + t, top, :], q3_s[qb * QT + t, bot, :]], axis=0)
             for t in range(QT)], axis=1)
        return jnp.where(((rows - lo) & 127) < DH, qt, jnp.uint32(0))

    def qprep(h, qb):
        qms[qb][0] = masked_q(h, qb)

    def k_rows(kb, k0, n):
        return k_s[kb, k0 // 2:(k0 + n) // 2, :]

    def gen(h, kt):
        _, _, lo, kb = head_geom(h)
        kx = pltpu.bitcast(k_rows(kb, (NC - 1 - kt) * TK, TK), bf16).astype(f32)
        kx = pltpu.roll(kx, (128 - lo) % 128, axis=1)
        for d in range(DH):
            kops[kt][d] = jnp.broadcast_to(kx[:, d:d + 1], (TK, 128))

    def ln_chunk(i):
        xn_s[i * XC:(i + 1) * XC, :] = _layernorm(
            x_s[i * XC:(i + 1) * XC, :].astype(f32)).astype(bf16)

    lane = lax.broadcasted_iota(jnp.int32, (XC // 2, 128), 1)

    def k_part(i, b0, b1):
        k = jnp.dot(xn_s[i * XC:(i + 1) * XC, :], wk_s[:, b0 * 128:b1 * 128],
                    preferred_element_type=f32).astype(bf16)
        k = pltpu.bitcast(k, jnp.uint32)
        r = slice(i * XC // 2, (i + 1) * XC // 2)
        for b in range(b0, b1):
            kb = k[:, (b - b0) * 128:(b - b0 + 1) * 128]
            k_s[b, r, :] = kb
            if b < NB - 1:
                pltpu.store(k_s.at[NB + b, r, :], kb, mask=lane >= 64)
            if b > 0:
                pltpu.store(k_s.at[NB + b - 1, r, :], kb, mask=lane < 64)

    def k_lo(i):
        k_part(i, 0, 2)

    def k_hi(i):
        k_part(i, 2, NB)

    def k_all(i):
        k_part(i, 0, NB)

    def proj(i, carry):
        r0 = pl.multiple_of(i * TR1, TR1)
        qv = lax.dot_general(wqvt_s[...], xn_s[pl.ds(r0, TR1), :],
                             (((1,), (1,)), ((), ())), preferred_element_type=f32)
        for t in range(TR1 // 128):
            q = qv[:D, t * 128:(t + 1) * 128] * QSCALE
            q3_s[i * (TR1 // 128) + t] = pltpu.bitcast(q.astype(bf16), jnp.uint32)
            qz = jnp.concatenate([q, jnp.zeros((16, 128), f32)], axis=0)
            for h in range(H):
                q4_s[i * (TR1 // 128) + t, h * QR:(h + 1) * QR, :] = qz[h * DH:h * DH + QR]
        for h in range(H):
            vt_s[h * VR:h * VR + DH, pl.ds(r0, TR1)] = qv[D + h * DH:D + (h + 1) * DH]
        return carry

    zacc_s[...] = jnp.zeros(zacc_s.shape, f32)
    pcar_s[...] = jnp.ones(pcar_s.shape, f32)
    acar_s[...] = jnp.zeros(acar_s.shape, f32)
    bad_s[...] = jnp.zeros(bad_s.shape, f32)
    sub = lax.broadcasted_iota(jnp.int32, (8, S), 0)
    tail_rows = jnp.where(sub == DH - 16, 1.0, 0.0).astype(f32)
    for h in range(H):
        vt_s[h * VR + 16:h * VR + 24, :] = tail_rows

    x_copy(0).wait()
    x_copy(1).start()
    ln_chunk(0)
    wk_copy.wait()
    x_copy(7).start()
    x_copy(6).start()
    k_lo(0)
    x_copy(1).wait()
    k_hi(0)
    ln_chunk(1)
    k_lo(1)
    x_copy(7).wait()
    x_copy(6).wait()
    for i in (5, 4, 3, 2):
        x_copy(i).start()
    k_hi(1)
    ln_chunk(7)
    k_all(7)
    ln_chunk(6)
    k_lo(6)
    for i in (5, 4, 3, 2):
        x_copy(i).wait()
    wq_copy.start()
    wv_copy.start()
    k_hi(6)
    ln_chunk(5)
    k_all(5)
    for kt in range(NK):
        gen(0, kt)
    ln_chunk(4)
    k_all(4)
    ln_chunk(3)
    k_lo(3)
    wq_copy.wait()
    wv_copy.wait()
    for c in late_copies:
        c.start()
    k_hi(3)
    ln_chunk(2)
    k_all(2)
    wqvt_s[0:D, :] = wq_s[...].T
    wqvt_s[D:2 * D, :] = wv_s[...].T
    lax.fori_loop(0, S // TR1, proj, None)
    qprep(0, 0)

    def vtile(h, n):
        kt, t = TILES[n]
        z = (_zero_after(h, 2) + n) >> 10
        qrow = pl.multiple_of((h + z) * QR, QR)
        acc = None
        for d in range(DH):
            q = jnp.broadcast_to(q4_s[t, pl.ds(qrow + d, 1), :], (8, 128))
            term = kops[kt][z + d].reshape(TK // 8, 8, 128) * q[None]
            acc = term if acc is None else acc + term
        pb, o = (kops[DLINE[n]], DH) if n in DLINE else (pbs[n % NPB], 0)
        pb[o] = jnp.exp2(acc).reshape(TK, 128)
        vt = vt_s[pl.ds(pl.multiple_of(h * VR, 8), VR), (NC - 1 - kt) * TK:(NC - kt) * TK]
        return jnp.dot(vt, pb[o + z], preferred_element_type=f32)

    def fin(h, qb, acc):
        l = acc[DH:DH + 1, :]
        ot_s[pl.ds(pl.multiple_of(h * VR, 8), VR), qb * TQ:(qb + 1) * TQ] = acc * (1.0 / l)
        ok = jnp.abs(acc) <= ACC_HI
        bad = jnp.max(jnp.where(ok, 0.0, 1.0).reshape(VR // 8, 8, TQ), axis=0)
        badl = jnp.where((l >= L_LO) & (l <= L_HI), 0.0, 1.0)
        bad_s[qb] = jnp.maximum(bad_s[qb], jnp.maximum(bad, badl))

    def carried(hp):
        vt = vt_s[pl.ds(pl.multiple_of(hp * VR, 8), VR), (NCA[-1] - 1) * TK:NCA[-1] * TK]
        r = jnp.dot(vt, pcar_s[...], preferred_element_type=f32)
        fin(hp, NQ - 1, acar_s[...] + r)

    def head(h, carry):
        kb0, hp = carry
        _, _, _, kb = head_geom(h)
        hn = jnp.minimum(h + 1, H - 1)
        vr0 = pl.multiple_of(h * VR, 8)
        pend = []
        vres = []
        accs = [None] * NQ

        def pv(qb, c, p):
            vt = vt_s[pl.ds(vr0, VR), c * TK:(c + 1) * TK]
            r = jnp.dot(vt, p, preferred_element_type=f32)
            accs[qb] = (zacc_s[qb] if accs[qb] is None else accs[qb]) + r

        def total(qb):
            acc = accs[qb]
            for kt in range(NKS[qb]):
                acc = acc + jnp.concatenate(
                    [vres[TILES.index((kt, qb * QT + t))] for t in range(QT)], axis=1)
            return acc

        for qb in range(1, NQ):
            qprep(h, qb)
        for slot in range(NSL):
            qb, c = SLOTS[slot]
            kc = pltpu.bitcast(jnp.concatenate(
                [k_rows(kb0 if slot == 0 else kb, c * TK + 16 * i, 16)
                 for i in reversed(range(8))], axis=0), bf16)
            zq = 0 if slot == 0 else (_zero_after(h, 1) + slot) >> 10
            w = pltpu.bitcast(qms[qb][zq], bf16)
            e = jnp.exp2(jnp.dot(kc, w, preferred_element_type=f32))
            pend.append((qb, c, jnp.concatenate(
                [e[16 * i:16 * (i + 1)] for i in reversed(range(8))], axis=0)))
            if slot == 0:
                carried(hp)
            else:
                pv(*pend.pop(0))
            target = min(NVT, max(0, slot + 1 - V_LATE) * NVT // (NSL - V_LATE - V_EARLY))
            while len(vres) < target:
                vres.append(vtile(h, len(vres)))
                n = len(vres)
                if n == NVT or TILES[n][0] != TILES[n - 1][0]:
                    gen(hn, TILES[n - 1][0])
        pcar_s[...] = pend.pop(0)[2]
        acar_s[...] = total(NQ - 1)
        for qb in range(NQ - 1):
            fin(h, qb, total(qb))
        qprep(hn, 0)
        return head_geom(hn, 0)[3], h

    def out_copy(i, r0=None, n=TR3):
        if r0 is None:
            r0 = pl.multiple_of(i * TR3, TR3)
        return pltpu.make_async_copy(out_s.at[pl.ds(r0, n), :],
                                     out_hbm.at[0, pl.ds(r0, n), :], sems.at[SEM_OUT + i])

    LAST = ((NT3 - 1, S - TR3, TR3 - TAIL), (NT3, S - TAIL, TAIL))

    def attn_out(i):
        r0 = pl.multiple_of(i * TR3, TR3)
        ot = jnp.concatenate(
            [ot_s[h * VR:h * VR + DH, pl.ds(r0, TR3)] for h in range(H)], axis=0)
        o = ot.T.astype(bf16)
        attn = jnp.dot(o, wo_s[...], preferred_element_type=f32)
        hres = x_s[pl.ds(r0, TR3), :].astype(f32) + attn
        hres_s[pl.ds(r0, TR3), :] = hres
        hn_s[pl.ds(r0, TR3), :] = _layernorm(hres).astype(bf16)

    def ffn(i, with_next):
        r0 = pl.multiple_of(i * TR3, TR3)
        u = jnp.dot(hn_s[pl.ds(r0, TR3), :], w1_s[...],
                    preferred_element_type=f32) + b1f_s[0:1, :]
        u = jax.nn.gelu(u, approximate=True).astype(bf16)
        if with_next:
            attn_out(i + 1)
            hres = hres_s[pl.ds(r0, TR3), :] + b2f_s[0:1, :]
            y = jnp.dot(u, w2_s[...], preferred_element_type=f32)
            out_s[pl.ds(r0, TR3), :] = (hres + y).astype(bf16)
            out_copy(i).start()
        else:
            hres = hres_s[pl.ds(r0, TR3), :] + b2f_s[0:1, :]
            for j, a, n in LAST:
                r = slice(a - (S - TR3), a - (S - TR3) + n)
                y = jnp.dot(u[r], w2_s[...], preferred_element_type=f32)
                out_s[a:a + n, :] = (hres[r] + y).astype(bf16)
                out_copy(j, a, n).start()

    lax.fori_loop(0, H, head, (jnp.int32(0), jnp.int32(H - 1)))
    for c in late_copies:
        c.wait()
    b1f_s[...] = jnp.broadcast_to(b1_s[...].astype(f32).reshape(1, F), (8, F))
    b2f_s[...] = jnp.broadcast_to(b2_s[...].astype(f32).reshape(1, D), (8, D))
    carried(H - 1)
    attn_out(0)

    @pl.when(jnp.max(bad_s[...]) > 0.0)
    def _():
        def item(t, carry):
            h = t // NQ
            qb = t % NQ
            _, _, _, kb = head_geom(h)
            qm = pltpu.bitcast(masked_q(h, qb), bf16)
            vr0 = pl.multiple_of(h * VR, 8)
            mrun = None
            for c in range(NC):
                kc = pltpu.bitcast(k_rows(kb, c * TK, TK), bf16)
                s = jnp.dot(kc, qm, preferred_element_type=f32)
                sbuf[c * TK:(c + 1) * TK, :] = s
                mc = jnp.max(s.reshape(TK // 8, 8, TQ), axis=0)
                mrun = mc if mrun is None else jnp.maximum(mrun, mc)
            m = jnp.max(mrun, axis=0, keepdims=True)
            acc = None
            for c in range(NC):
                p = jnp.exp2(sbuf[c * TK:(c + 1) * TK, :] - m)
                r = jnp.dot(vt_s[pl.ds(vr0, VR), c * TK:(c + 1) * TK], p,
                            preferred_element_type=f32)
                acc = r if acc is None else acc + r
            l = acc[DH:DH + 1, :]
            ot_s[pl.ds(vr0, VR), pl.ds(pl.multiple_of(qb * TQ, TQ), TQ)] = acc * (1.0 / l)
            return carry

        lax.fori_loop(0, H * NQ, item, None)
        attn_out(0)

    def tail(i, c):
        ffn(i, True)
        return c

    lax.fori_loop(0, NT3 - 1, tail, None)
    ffn(NT3 - 1, False)
    for i in range(NT3 - 1):
        out_copy(i).wait()
    for j, a, n in LAST:
        out_copy(j, a, n).wait()


@jax.jit
def pallas_sequential_preLN__softmax_full_mha__dense_activation_gelu__prompt_kernel(
    A_x: jax.Array,
    A_wqkv: jax.Array,
    A_wo: jax.Array,
    B_x: jax.Array,
    B_w1: jax.Array,
    B_b1: jax.Array,
    B_w2: jax.Array,
    B_b2: jax.Array,
):
    del B_x
    bf16 = jnp.bfloat16
    f32 = jnp.float32
    u32 = jnp.uint32
    any_spec = pl.BlockSpec(memory_space=pl.ANY)
    return pl.pallas_call(
        _kernel,
        out_shape=jax.ShapeDtypeStruct(A_x.shape, A_x.dtype),
        in_specs=[any_spec] * 7,
        out_specs=any_spec,
        scratch_shapes=[
            pltpu.VMEM((S, D), bf16),
            pltpu.VMEM((D, D), bf16),
            pltpu.VMEM((D, D), bf16),
            pltpu.VMEM((D, D), bf16),
            pltpu.VMEM((D, D), bf16),
            pltpu.VMEM((D, F), bf16),
            pltpu.VMEM((F, D), bf16),
            pltpu.VMEM((2 * D, D), bf16),
            pltpu.VMEM((S, D), bf16),
            pltpu.VMEM((2 * NB - 1, S // 2, 128), u32),
            pltpu.VMEM((NQT, D // 2, 128), u32),
            pltpu.VMEM((NQT, H * QR, 128), f32),
            pltpu.VMEM((H * VR, S), f32),
            pltpu.VMEM((H * VR, S), f32),
            pltpu.VMEM((S, TQ), f32),
            pltpu.VMEM((DH + 1, TK, 128), f32),
            pltpu.VMEM((DH + 1, TK, 128), f32),
            pltpu.VMEM((DH + 1, TK, 128), f32),
        ] + [pltpu.VMEM((1, TK, 128), f32)] * NPB
          + [pltpu.VMEM((1, 64, TQ), u32)] * NQ + [
            pltpu.VMEM((NQ, VR, TQ), f32),
            pltpu.VMEM((TK, TQ), f32),
            pltpu.VMEM((VR, TQ), f32),
            pltpu.VMEM((NQ, 8, TQ), f32),
            pltpu.VMEM((S, D), f32),
            pltpu.VMEM((S, D), bf16),
            pltpu.VMEM((S, D), bf16),
            pltpu.VMEM((8, F), f32),
            pltpu.VMEM((8, D), f32),
            pltpu.VMEM((F,), bf16),
            pltpu.VMEM((D,), bf16),
            pltpu.SemaphoreType.DMA((NSEM,)),
        ],
        compiler_params=pltpu.CompilerParams(vmem_limit_bytes=100 * 1024 * 1024),
    )(A_x, A_wqkv, A_wo, B_w1, B_b1, B_w2, B_b2)
```
